```python
import os as _os
_os.environ.setdefault("JAX_PLATFORMS", "cpu")
import jax
import jax.numpy as jnp

def _softmax(x, axis=-1):
    return jax.nn.softmax(x, axis=axis)
def _gelu(x):
    return jax.nn.gelu(x, approximate=True)
def _silu(x):
    return jax.nn.silu(x)
def _sigmoid(x):
    return jax.nn.sigmoid(x)
def _layernorm(x, axis=-1, eps=1e-5):
    m = jnp.mean(x, axis=axis, keepdims=True)
    v = jnp.var(x, axis=axis, keepdims=True)
    return (x - m) / jnp.sqrt(v + eps)
def _scatter_add(tgt, idx, src, axis=0):
    return tgt.at[idx].add(src)
def _segment_sum(src, seg, n):
    return jax.ops.segment_sum(src, seg, n)
class _Rng:
    def __init__(self, key):
        self._k = key
    def _next(self):
        self._k, sub = jax.random.split(self._k)
        return sub
    def normal(self, shape):
        return jax.random.normal(self._next(), shape, dtype=jnp.bfloat16)
    def randint(self, lo, hi, shape):
        return jax.random.randint(self._next(), shape, lo, hi, dtype=jnp.int32)
    def uniform(self, shape, lo=0.0, hi=1.0):
        return jax.random.uniform(self._next(), shape, jnp.bfloat16, lo, hi)
    def permutation(self, n):
        return jax.random.permutation(self._next(), n)


kernel_name = 'parallel_sum__sliding_block_cached__dense_activation_mish__decode'

def setup_inputs():
    _rng = _Rng(jax.random.key(int.from_bytes(__import__("os").urandom(4), "little")))
    _w = (lambda a: (lambda t: t.astype(jnp.bfloat16) if jnp.issubdtype(t.dtype, jnp.floating) else t)(jnp.asarray(a)))
    def _A_setup():
        B, Sq, D = 2, 1, 512
        Hq, Hkv, Sk, Dh = 32, 8, 32768, 128
        assert Hq % Hkv == 0, (Hq, Hkv)
        return {
            "x": _w((lambda *s: _rng.normal(s) * 0.05)(B, Sq, D)),
            "k_cache": _w((lambda *s: _rng.normal(s) * 0.8)(B, Hkv, Sk, Dh)),
            "v_cache": _w((lambda *s: _rng.normal(s) * 0.8)(B, Hkv, Sk, Dh)),
            "wq": _w((lambda *s: _rng.normal(s) * 0.8)(D, Hq * Dh) * (D ** -0.5)),
            "wo": _w((lambda *s: _rng.normal(s) * 0.8)(Hq * Dh, D) * ((Hq * Dh) ** -0.5)),
        }
    _A_in = _A_setup()

    def _B_setup():
        B, S, D, F = 2, 1, 512, 1792
        return {
            "x": _w((lambda *s: _rng.normal(s) * 0.05)(B, S, D)),
            "w1": _w((lambda *s: _rng.normal(s) * 0.4)(D, F) * (D ** -0.5)),
            "b1": _w((lambda *s: _rng.normal(s) * 0.05)(F)),
            "w2": _w((lambda *s: _rng.normal(s) * 0.05)(F, D) * (F ** -0.5)),
        }
    _B_in = _B_setup()

    return {
        "A_x": _A_in["x"],
        "A_k_cache": _A_in["k_cache"],
        "A_v_cache": _A_in["v_cache"],
        "A_wq": _A_in["wq"],
        "A_wo": _A_in["wo"],
        "B_x": _B_in["x"],
        "B_w1": _B_in["w1"],
        "B_b1": _B_in["b1"],
        "B_w2": _B_in["w2"],
    }

def reference(A_x, A_k_cache, A_v_cache, A_wq, A_wo, B_x, B_w1, B_b1, B_w2):
    def _A_ref(x, k_cache, v_cache, wq, wo):
        B, Sq, D = x.shape
        Hq, Dh = 32, 128
        Hkv, Sk = k_cache.shape[1], k_cache.shape[2]
        W = min(4096, max(256, Sk // 4))
        rep = Hq // Hkv
        q = (lambda x, *d: x.transpose(*d))((x @ wq).reshape(B, Sq, Hq, Dh), 0, 2, 1, 3)
        k = jnp.repeat(k_cache[:, :, Sk - W:, :], rep, axis=1)
        v = jnp.repeat(v_cache[:, :, Sk - W:, :], rep, axis=1)
        scores = jnp.einsum("bhqd,bhkd->bhqk", q, k) * (Dh ** -0.5)
        p = _softmax(scores, axis=-1)
        o = jnp.einsum("bhqk,bhkd->bhqd", p, v)
        return (lambda x, *d: x.transpose(*d))(o, 0, 2, 1, 3).reshape(B, Sq, Hq * Dh) @ wo

    def _B_ref(x, w1, b1, w2):
        h = jnp.einsum("bsd,df->bsf", x, w1) + b1
        sp = jnp.log1p(jnp.exp(-jnp.abs(h))) + jnp.where(h > 0, h, jnp.zeros_like(h))
        act = h * jnp.tanh(sp)
        return jnp.einsum("bsf,fd->bsd", act, w2)

    x = A_x
    xn = _layernorm(x, axis=-1)
    return x + _A_ref(xn, A_k_cache, A_v_cache, A_wq, A_wo) + _B_ref(xn, B_w1, B_b1, B_w2)
```

```python
import jax
import jax.numpy as jnp
from jax import lax
import jax.experimental.pallas as pl
import jax.experimental.pallas.tpu as pltpu

HQ, DH = 32, 128
LN_EPS = 1e-5
_NT = (((1,), (1,)), ((), ()))


@jax.jit
def pallas_parallel_sum__sliding_block_cached__dense_activation_mish__decode_kernel(
    A_x: jax.Array,
    A_k_cache: jax.Array,
    A_v_cache: jax.Array,
    A_wq: jax.Array,
    A_wo: jax.Array,
    B_x: jax.Array,
    B_w1: jax.Array,
    B_b1: jax.Array,
    B_w2: jax.Array,
):
    del B_x
    B, Sq, D = A_x.shape
    HKV, SK = A_k_cache.shape[1], A_k_cache.shape[2]
    F = B_w1.shape[1]
    W = min(4096, max(256, SK // 4))
    REP = HQ // HKV
    R = B * REP
    assert (B, Sq, R) == (2, 1, 8)
    w2_chunks = (F - 768, 512, 128, 128)
    w2_offs = [sum(w2_chunks[:i]) for i in range(len(w2_chunks))]

    def kernel(x_hbm, b1_hbm, k_hbm, v_hbm, wq_hbm, wo_hbm, w1_hbm, w2_hbm, o_ref,
               x_v, b1_v, k_v, v_v, wq_v, wo_v, w1_v, w2_v, q_s, p_s, l_s, o_s, sems):
        cq = pltpu.make_async_copy(wq_hbm, wq_v, sems.at[0])
        cx = pltpu.make_async_copy(x_hbm, x_v, sems.at[0])
        cb = pltpu.make_async_copy(b1_hbm, b1_v, sems.at[0])
        c1 = pltpu.make_async_copy(w1_hbm, w1_v, sems.at[0])
        ck = pltpu.make_async_copy(k_hbm.at[:, :, pl.ds(SK - W, W), :], k_v, sems.at[1])
        cv = pltpu.make_async_copy(v_hbm.at[:, :, pl.ds(SK - W, W), :], v_v, sems.at[2])
        co = pltpu.make_async_copy(wo_hbm, wo_v, sems.at[3])
        c2 = [
            pltpu.make_async_copy(w2_hbm.at[pl.ds(o, n), :], w2_v.at[pl.ds(o, n), :], sems.at[4 + i])
            for i, (o, n) in enumerate(zip(w2_offs, w2_chunks))
        ]
        for c in (cq, cx, cb, c1, ck, cv, co, *c2):
            c.start()

        for c in (cq, cx, cb, c1):
            c.wait()
        xx = x_v[...].astype(jnp.float32)
        row = lax.broadcasted_iota(jnp.int32, (R, D), 0)
        x = jnp.where(row % B == 0, jnp.broadcast_to(xx[0:1], (R, D)), jnp.broadcast_to(xx[1:2], (R, D)))
        xc = x - jnp.mean(x, axis=-1, keepdims=True)
        var = jnp.mean(xc * xc, axis=-1, keepdims=True)
        xn = (xc / jnp.sqrt(var + LN_EPS)).astype(jnp.bfloat16)

        r128 = lax.broadcasted_iota(jnp.int32, (R, DH), 0)

        def q_body(g, carry):
            cols = pl.ds(pl.multiple_of(g * REP * DH, REP * DH), REP * DH)
            q = jnp.dot(xn, wq_v[:, cols], preferred_element_type=jnp.float32)
            qg = q[:, :DH]
            for r in range(1, REP):
                qg = jnp.where(r128 // B == r, q[:, r * DH:(r + 1) * DH], qg)
            q_s[g] = qg
            return carry

        lax.fori_loop(0, HKV, q_body, 0)

        h = jnp.dot(xn, w1_v[...], preferred_element_type=jnp.float32)
        h = h + b1_v[...].astype(jnp.float32).reshape(1, F)
        sp = jnp.log1p(jnp.exp(-jnp.abs(h))) + jnp.where(h > 0, h, 0.0)
        act = (h * jnp.tanh(sp)).astype(jnp.bfloat16)

        ck.wait()

        def s_body(g, carry):
            qg = q_s[g].astype(jnp.bfloat16)
            s0 = lax.dot_general(qg, k_v[0, g], _NT, preferred_element_type=jnp.float32)
            s1 = lax.dot_general(qg, k_v[1, g], _NT, preferred_element_type=jnp.float32)
            rr = lax.broadcasted_iota(jnp.int32, (R, W), 0)
            s = jnp.where(rr % B == 0, s0, s1) * (DH ** -0.5)
            p = jnp.exp(s - jnp.max(s, axis=-1, keepdims=True))
            l_s[g] = jnp.broadcast_to(jnp.sum(p, axis=-1, keepdims=True), (R, DH))
            p_s[g] = p
            return carry

        lax.fori_loop(0, HKV, s_body, 0)

        cv.wait()

        def o_body(g, carry):
            pb = p_s[g].astype(jnp.bfloat16)
            o0 = jnp.dot(pb, v_v[0, g], preferred_element_type=jnp.float32)
            o1 = jnp.dot(pb, v_v[1, g], preferred_element_type=jnp.float32)
            o_s[g] = jnp.where(r128 % B == 0, o0, o1) / l_s[g]
            return carry

        lax.fori_loop(0, HKV, o_body, 0)

        co.wait()

        def w_body(g, acc):
            og = o_s[g]
            lhs = jnp.concatenate(
                [jnp.where(r128 // B == r, og, 0.0) for r in range(REP)], axis=1
            ).astype(jnp.bfloat16)
            rows = pl.ds(pl.multiple_of(g * REP * DH, REP * DH), REP * DH)
            return acc + jnp.dot(lhs, wo_v[rows, :], preferred_element_type=jnp.float32)

        a = lax.fori_loop(0, HKV, w_body, jnp.zeros((R, D), jnp.float32))
        a = a + pltpu.roll(a, 2, axis=0)
        a = a + pltpu.roll(a, 4, axis=0)
        acc = x + a
        for c, o, n in zip(c2, w2_offs, w2_chunks):
            c.wait()
            acc = acc + jnp.dot(act[:, o:o + n], w2_v[pl.ds(o, n), :], preferred_element_type=jnp.float32)
        o_ref[...] = acc[0:B].astype(o_ref.dtype)

    hbm = pl.BlockSpec(memory_space=pltpu.HBM)
    out = pl.pallas_call(
        kernel,
        in_specs=[hbm] * 8,
        out_specs=pl.BlockSpec(memory_space=pltpu.VMEM),
        out_shape=jax.ShapeDtypeStruct((B, D), A_x.dtype),
        scratch_shapes=[
            pltpu.VMEM((B, D), A_x.dtype),
            pltpu.VMEM((F,), B_b1.dtype),
            pltpu.VMEM((B, HKV, W, DH), A_k_cache.dtype),
            pltpu.VMEM((B, HKV, W, DH), A_v_cache.dtype),
            pltpu.VMEM((D, HQ * DH), A_wq.dtype),
            pltpu.VMEM((HQ * DH, D), A_wo.dtype),
            pltpu.VMEM((D, F), B_w1.dtype),
            pltpu.VMEM((F, D), B_w2.dtype),
            pltpu.VMEM((HKV, R, DH), jnp.float32),
            pltpu.VMEM((HKV, R, W), jnp.float32),
            pltpu.VMEM((HKV, R, DH), jnp.float32),
            pltpu.VMEM((HKV, R, DH), jnp.float32),
            pltpu.SemaphoreType.DMA((4 + len(w2_chunks),)),
        ],
        compiler_params=pltpu.CompilerParams(vmem_limit_bytes=100 * 1024 * 1024),
    )(A_x.reshape(B, D), B_b1, A_k_cache, A_v_cache, A_wq, A_wo, B_w1, B_w2)
    return out.reshape(B, Sq, D)
```

```python
import jax
import jax.numpy as jnp
from jax import lax
import jax.experimental.pallas as pl
import jax.experimental.pallas.tpu as pltpu

HQ, DH = 32, 128
LN_EPS = 1e-5
SUBLANES, LANES = 8, 128
_NT = (((1,), (1,)), ((), ()))
_W2_LAST_MXU = 384
_W2_VPU = (144, 64, 32, 16)


@jax.jit
def pallas_parallel_sum__sliding_block_cached__dense_activation_mish__decode_kernel(
    A_x: jax.Array,
    A_k_cache: jax.Array,
    A_v_cache: jax.Array,
    A_wq: jax.Array,
    A_wo: jax.Array,
    B_x: jax.Array,
    B_w1: jax.Array,
    B_b1: jax.Array,
    B_w2: jax.Array,
):
    del B_x
    B, Sq, D = A_x.shape
    HKV, SK = A_k_cache.shape[1], A_k_cache.shape[2]
    F = B_w1.shape[1]
    W = min(4096, max(256, SK // 4))
    REP = HQ // HKV
    R = B * REP
    assert (B, Sq, R) == (2, 1, SUBLANES)
    GW = REP * DH

    n_vpu = sum(_W2_VPU)
    chunks = (F - n_vpu - _W2_LAST_MXU, _W2_LAST_MXU) + _W2_VPU
    offs = tuple(sum(chunks[:i]) for i in range(len(chunks)))
    n_mxu_chunks = len(chunks) - len(_W2_VPU)
    assert chunks[0] > 0 and chunks[0] % LANES == 0 and n_vpu % LANES == 0
    f32, mxu = jnp.float32, A_wq.dtype

    def kernel(x_hbm, b1_hbm, k_hbm, v_hbm, wq_hbm, wo_hbm, w1_hbm, w2_hbm, o_ref,
               x_v, b1_v, k_v, v_v, wq_v, wo_v, w1_v, w2_v, q_s, p_s, l_s, o_s, a_s):

        def vpu_step(i, parts):
            o, n = offs[i], chunks[i]
            w = w2_v[pl.ds(o, n), :].astype(f32)
            out = []
            for b in range(B):
                a = a_s[b, pl.ds(o - (F - n_vpu), n), :]
                prod = w * jnp.concatenate([a] * (D // LANES), axis=1)
                out.append(parts[b] + jnp.sum(prod.reshape(n // SUBLANES, SUBLANES, D), axis=0))
            return out

        def stream(sems):
            cq = pltpu.make_async_copy(wq_hbm, wq_v, sems.at[0])
            cx = pltpu.make_async_copy(x_hbm, x_v, sems.at[0])
            cb = pltpu.make_async_copy(b1_hbm, b1_v, sems.at[0])
            c1 = pltpu.make_async_copy(w1_hbm, w1_v, sems.at[0])
            ck = pltpu.make_async_copy(k_hbm.at[:, :, pl.ds(SK - W, W), :], k_v, sems.at[1])
            cv = pltpu.make_async_copy(v_hbm.at[:, :, pl.ds(SK - W, W), :], v_v, sems.at[2])
            co = pltpu.make_async_copy(wo_hbm, wo_v, sems.at[3])
            c2 = [
                pltpu.make_async_copy(
                    w2_hbm.at[pl.ds(o, n), :], w2_v.at[pl.ds(o, n), :], sems.at[4 + i])
                for i, (o, n) in enumerate(zip(offs, chunks))
            ]
            for c in (cq, cx, cb, c1, ck, cv, co, *c2):
                c.start()

            for c in (cq, cx, cb, c1):
                c.wait()

            row = lax.broadcasted_iota(jnp.int32, (R, D), 0)
            x2 = x_v[...].astype(f32)
            x = jnp.where(row % B == 0, jnp.broadcast_to(x2[0:1], (R, D)),
                          jnp.broadcast_to(x2[1:2], (R, D)))
            xc = x - jnp.mean(x, axis=-1, keepdims=True)
            var = jnp.mean(xc * xc, axis=-1, keepdims=True)
            xn = (xc / jnp.sqrt(var + LN_EPS)).astype(mxu)

            row_h = lax.broadcasted_iota(jnp.int32, (R, DH), 0)

            def q_body(g, carry):
                cols = pl.ds(pl.multiple_of(g * GW, GW), GW)
                q = jnp.dot(xn, wq_v[:, cols], preferred_element_type=f32)
                qg = q[:, :DH]
                for r in range(1, REP):
                    qg = jnp.where(row_h // B == r, q[:, r * DH:(r + 1) * DH], qg)
                q_s[g] = qg
                return carry

            lax.fori_loop(0, HKV, q_body, 0)

            h = jnp.dot(xn, w1_v[...], preferred_element_type=f32)
            h = h + b1_v[...].astype(f32).reshape(1, F)
            sp = jnp.log1p(jnp.exp(-jnp.abs(h))) + jnp.where(h > 0, h, 0.0)
            act = (h * jnp.tanh(sp)).astype(mxu)
            act_vpu = act[:, F - n_vpu:].astype(f32)
            for b in range(B):
                a_s[b] = jnp.broadcast_to(act_vpu[b:b + 1], (LANES, n_vpu)).T

            ck.wait()

            def s_body(g, carry):
                qg = q_s[g].astype(mxu)
                s0 = lax.dot_general(qg, k_v[0, g], _NT, preferred_element_type=f32)
                s1 = lax.dot_general(qg, k_v[1, g], _NT, preferred_element_type=f32)
                row_w = lax.broadcasted_iota(jnp.int32, (R, W), 0)
                s = jnp.where(row_w % B == 0, s0, s1) * (DH ** -0.5)
                p = jnp.exp(s - jnp.max(s, axis=-1, keepdims=True))
                l_s[g] = jnp.broadcast_to(jnp.sum(p, axis=-1, keepdims=True), (R, DH))
                p_s[g] = p
                return carry

            lax.fori_loop(0, HKV, s_body, 0)

            cv.wait()

            def o_body(g, carry):
                p = p_s[g].astype(mxu)
                o0 = jnp.dot(p, v_v[0, g], preferred_element_type=f32)
                o1 = jnp.dot(p, v_v[1, g], preferred_element_type=f32)
                o_s[g] = jnp.where(row_h % B == 0, o0, o1) / l_s[g]
                return carry

            lax.fori_loop(0, HKV, o_body, 0)

            co.wait()

            def w_body(g, acc):
                og = o_s[g]
                lhs = jnp.concatenate(
                    [jnp.where(row_h // B == r, og, 0.0) for r in range(REP)], axis=1)
                rows = pl.ds(pl.multiple_of(g * GW, GW), GW)
                return acc + jnp.dot(lhs.astype(mxu), wo_v[rows, :], preferred_element_type=f32)

            attn = lax.fori_loop(0, HKV, w_body, jnp.zeros((R, D), f32))
            attn = attn + pltpu.roll(attn, 2, axis=0)
            attn = attn + pltpu.roll(attn, 4, axis=0)
            acc = x + attn

            for i in range(n_mxu_chunks):
                o, n = offs[i], chunks[i]
                c2[i].wait()
                acc = acc + jnp.dot(act[:, o:o + n], w2_v[pl.ds(o, n), :],
                                    preferred_element_type=f32)
            parts = [jnp.where(row == b, acc, 0.0) for b in range(B)]
            for i in range(n_mxu_chunks, len(chunks) - 1):
                c2[i].wait()
                parts = vpu_step(i, parts)
            c2[-1].wait()
            return parts

        parts = pl.run_scoped(stream, pltpu.SemaphoreType.DMA((4 + len(chunks),)))
        parts = vpu_step(len(chunks) - 1, parts)
        out = jnp.concatenate([jnp.sum(p, axis=0, keepdims=True) for p in parts], axis=0)
        o_ref[...] = out.astype(o_ref.dtype)

    hbm = pl.BlockSpec(memory_space=pltpu.HBM)
    out = pl.pallas_call(
        kernel,
        in_specs=[hbm] * 8,
        out_specs=pl.BlockSpec(memory_space=pltpu.VMEM),
        out_shape=jax.ShapeDtypeStruct((B, D), A_x.dtype),
        scratch_shapes=[
            pltpu.VMEM((B, D), A_x.dtype),
            pltpu.VMEM((F,), B_b1.dtype),
            pltpu.VMEM((B, HKV, W, DH), A_k_cache.dtype),
            pltpu.VMEM((B, HKV, W, DH), A_v_cache.dtype),
            pltpu.VMEM((D, HQ * DH), A_wq.dtype),
            pltpu.VMEM((HQ * DH, D), A_wo.dtype),
            pltpu.VMEM((D, F), B_w1.dtype),
            pltpu.VMEM((F, D), B_w2.dtype),
            pltpu.VMEM((HKV, R, DH), f32),
            pltpu.VMEM((HKV, R, W), f32),
            pltpu.VMEM((HKV, R, DH), f32),
            pltpu.VMEM((HKV, R, DH), f32),
            pltpu.VMEM((B, n_vpu, LANES), f32),
        ],
        compiler_params=pltpu.CompilerParams(vmem_limit_bytes=64 * 1024 * 1024),
    )(A_x.reshape(B, D), B_b1, A_k_cache, A_v_cache, A_wq, A_wo, B_w1, B_w2)
    return out.reshape(B, Sq, D)
```
